```python
import os as _os
_os.environ.setdefault("JAX_PLATFORMS", "cpu")
import jax
import jax.numpy as jnp

def _softmax(x, axis=-1):
    return jax.nn.softmax(x, axis=axis)
def _gelu(x):
    return jax.nn.gelu(x, approximate=True)
def _silu(x):
    return jax.nn.silu(x)
def _sigmoid(x):
    return jax.nn.sigmoid(x)
def _layernorm(x, axis=-1, eps=1e-5):
    m = jnp.mean(x, axis=axis, keepdims=True)
    v = jnp.var(x, axis=axis, keepdims=True)
    return (x - m) / jnp.sqrt(v + eps)
def _scatter_add(tgt, idx, src, axis=0):
    return tgt.at[idx].add(src)
def _segment_sum(src, seg, n):
    return jax.ops.segment_sum(src, seg, n)
class _Rng:
    def __init__(self, key):
        self._k = key
    def _next(self):
        self._k, sub = jax.random.split(self._k)
        return sub
    def normal(self, shape):
        return jax.random.normal(self._next(), shape, dtype=jnp.bfloat16)
    def randint(self, lo, hi, shape):
        return jax.random.randint(self._next(), shape, lo, hi, dtype=jnp.int32)
    def uniform(self, shape, lo=0.0, hi=1.0):
        return jax.random.uniform(self._next(), shape, jnp.bfloat16, lo, hi)
    def permutation(self, n):
        return jax.random.permutation(self._next(), n)


kernel_name = 'concat_heads__mha_block_cached__mha_block_cached__near_ridge'

def setup_inputs():
    _rng = _Rng(jax.random.key(int.from_bytes(__import__("os").urandom(4), "little")))
    _w = (lambda a: (lambda t: t.astype(jnp.bfloat16) if jnp.issubdtype(t.dtype, jnp.floating) else t)(jnp.asarray(a)))
    def _A_setup():
        B, Sq, D = 32, 32, 640
        H, Sk, Dh = 32, 32, 128
        return {
            "x": _w((lambda *s: _rng.normal(s) * 0.8)(B, Sq, D)),
            "k_cache": _w((lambda *s: _rng.normal(s) * 0.8)(B, H, Sk, Dh)),
            "v_cache": _w((lambda *s: _rng.normal(s) * 0.05)(B, H, Sk, Dh)),
            "wq": _w((lambda *s: _rng.normal(s) * 0.8)(D, H * Dh) * (D ** -0.5)),
            "wo": _w((lambda *s: _rng.normal(s) * 0.05)(H * Dh, D) * ((H * Dh) ** -0.5)),
        }
    _A_in = _A_setup()

    def _B_setup():
        B, Sq, D = 32, 32, 640
        H, Sk, Dh = 32, 32, 128
        return {
            "x": _w((lambda *s: _rng.normal(s) * 0.8)(B, Sq, D)),
            "k_cache": _w((lambda *s: _rng.normal(s) * 0.8)(B, H, Sk, Dh)),
            "v_cache": _w((lambda *s: _rng.normal(s) * 0.05)(B, H, Sk, Dh)),
            "wq": _w((lambda *s: _rng.normal(s) * 0.8)(D, H * Dh) * (D ** -0.5)),
            "wo": _w((lambda *s: _rng.normal(s) * 0.05)(H * Dh, D) * ((H * Dh) ** -0.5)),
        }
    _B_in = _B_setup()

    return {
        "A_x": _A_in["x"],
        "A_k_cache": _A_in["k_cache"],
        "A_v_cache": _A_in["v_cache"],
        "A_wq": _A_in["wq"],
        "A_wo": _A_in["wo"],
        "B_x": _B_in["x"],
        "B_k_cache": _B_in["k_cache"],
        "B_v_cache": _B_in["v_cache"],
        "B_wq": _B_in["wq"],
        "B_wo": _B_in["wo"],
    }

def reference(A_x, A_k_cache, A_v_cache, A_wq, A_wo, B_x, B_k_cache, B_v_cache, B_wq, B_wo):
    def _A_ref(x, k_cache, v_cache, wq, wo):
        B, Sq, D = x.shape
        H, Dh = 32, 128
        q = (lambda x, *d: x.transpose(*d))((x @ wq).reshape(B, Sq, H, Dh), 0, 2, 1, 3)
        scores = jnp.einsum("bhqd,bhkd->bhqk", q, k_cache) * (Dh ** -0.5)
        p = _softmax(scores, axis=-1)
        o = jnp.einsum("bhqk,bhkd->bhqd", p, v_cache)
        return (lambda x, *d: x.transpose(*d))(o, 0, 2, 1, 3).reshape(B, Sq, H * Dh) @ wo

    def _B_ref(x, k_cache, v_cache, wq, wo):
        B, Sq, D = x.shape
        H, Dh = 32, 128
        q = (lambda x, *d: x.transpose(*d))((x @ wq).reshape(B, Sq, H, Dh), 0, 2, 1, 3)
        scores = jnp.einsum("bhqd,bhkd->bhqk", q, k_cache) * (Dh ** -0.5)
        p = _softmax(scores, axis=-1)
        o = jnp.einsum("bhqk,bhkd->bhqd", p, v_cache)
        return (lambda x, *d: x.transpose(*d))(o, 0, 2, 1, 3).reshape(B, Sq, H * Dh) @ wo

    a = _A_ref(A_x, A_k_cache, A_v_cache, A_wq, A_wo)
    b = _B_ref(B_x, B_k_cache, B_v_cache, B_wq, B_wo)
    return jnp.concatenate([a, b], axis=-1)
```

```python
import functools
import jax
import jax.numpy as jnp
from jax import lax
import jax.experimental.pallas as pl
import jax.experimental.pallas.tpu as pltpu

B, SQ, D = 32, 32, 640
H, SK, DH = 32, 32, 128
M = B * SQ
HPG = 4
G = H // HPG
GW = HPG * DH
NSTEPS = 2 * G
SCALE = DH ** -0.5
NCH = 4
CB = B // NCH
CM = CB * SQ


def _kernel(xa, ka, va, wqa, woa, xb, kb, vb, wqb, wob, out_hbm,
            x_buf, wq_buf, k_buf, v_buf, wo_buf, q_scr, p_scr, o_scr, acc, out_buf,
            x_sem, wq_sem, k_sem, v_sem, wo_sem, out_sem, f_sem):
    s = pl.program_id(0)
    branch = s // G
    g = s % G
    slot = s % 2
    last_g = g == G - 1

    def copies(refs, gg, sl):
        k_h, v_h, wq_h, wo_h = refs
        return (
            pltpu.make_async_copy(wq_h.at[:, pl.ds(gg * GW, GW)], wq_buf.at[sl], wq_sem.at[sl]),
            pltpu.make_async_copy(k_h.at[:, pl.ds(gg * HPG, HPG)], k_buf.at[sl], k_sem.at[sl]),
            pltpu.make_async_copy(v_h.at[:, pl.ds(gg * HPG, HPG)], v_buf.at[sl], v_sem.at[sl]),
            pltpu.make_async_copy(wo_h.at[pl.ds(gg * GW, GW), :], wo_buf.at[sl], wo_sem.at[sl]),
        )

    def out_copy(br, c):
        return pltpu.make_async_copy(
            out_buf.at[br, pl.ds(c * CM, CM), :],
            out_hbm.at[pl.ds(c * CM, CM), pl.ds(br * D, D)],
            out_sem.at[br, c])

    def fx(c):
        return pltpu.make_async_copy(xa.at[pl.ds(c * (M // 2), M // 2), :],
                                     x_buf.at[0, pl.ds(c * (M // 2), M // 2), :], f_sem.at[c])

    refs_a = (ka, va, wqa, woa)
    refs_b = (kb, vb, wqb, wob)

    def step(first):
        cw_q, cw_k, cw_v, cw_o = copies(refs_a, 0, slot)
        if first:
            for cp in (fx(0), cw_q):
                cp.start()
            acc[...] = jnp.zeros_like(acc)
        else:
            @pl.when(s == G)
            def _():
                pltpu.make_async_copy(xb, x_buf.at[1], x_sem.at[0]).wait()

            cw_q.wait()
            cw_k.wait()
            cw_v.wait()
            cw_o.wait()

            nxt = s + 1

            @pl.when(nxt < G)
            def _():
                for c in copies(refs_a, nxt, 1 - slot):
                    c.start()

            @pl.when(jnp.logical_and(nxt >= G, nxt < NSTEPS))
            def _():
                for c in copies(refs_b, nxt - G, 1 - slot):
                    c.start()

            @pl.when(s == 1)
            def _():
                pltpu.make_async_copy(xb, x_buf.at[1], x_sem.at[0]).start()

        row = lax.broadcasted_iota(jnp.int32, (HPG * SQ, HPG * SK), 0) // SQ
        col = lax.broadcasted_iota(jnp.int32, (HPG * SQ, HPG * SK), 1) // SK
        mask = row == col

        def qproj(c):
            x = x_buf[branch, c * CM:(c + 1) * CM, :]
            for h in range(HPG):
                qh = jnp.dot(x, wq_buf[slot, :, h * DH:(h + 1) * DH], preferred_element_type=jnp.float32)
                q_scr[c * CB:(c + 1) * CB, h] = qh.astype(jnp.bfloat16).reshape(CB, SQ, DH)

        def scores(c):
            for b in range(c * CB, (c + 1) * CB):
                qs = q_scr[b].reshape(HPG * SQ, DH)
                ks = k_buf[slot, b].reshape(HPG * SK, DH)
                sc = lax.dot_general(qs, ks, (((1,), (1,)), ((), ())), preferred_element_type=jnp.float32)
                sc = jnp.where(mask, sc, -jnp.inf)
                m = jnp.max(sc, axis=1, keepdims=True)
                e = jnp.exp((sc - m) * SCALE)
                l = jnp.sum(e, axis=1, keepdims=True)
                r0 = pl.reciprocal(l, approx=True)
                r = r0 * (2.0 - l * r0)
                p_scr[b] = (e * r).astype(jnp.bfloat16)

        def pv(c):
            for b in range(c * CB, (c + 1) * CB):
                vs = v_buf[slot, b].reshape(HPG * SK, DH)
                o = jnp.dot(p_scr[b], vs, preferred_element_type=jnp.float32).astype(jnp.bfloat16)
                for h in range(HPG):
                    o_scr[b * SQ:(b + 1) * SQ, h * DH:(h + 1) * DH] = o[h * SQ:(h + 1) * SQ, :]

        def oproj(c):
            a = acc[c * CM:(c + 1) * CM, :] + jnp.dot(o_scr[c * CM:(c + 1) * CM, :], wo_buf[slot],
                                                      preferred_element_type=jnp.float32)
            if first:
                acc[c * CM:(c + 1) * CM, :] = a
            else:
                out_buf[branch, c * CM:(c + 1) * CM, :] = a.astype(jnp.bfloat16)
                acc[c * CM:(c + 1) * CM, :] = jnp.where(last_g, 0.0, a)

                @pl.when(last_g)
                def _():
                    out_copy(branch, c).start()

        if first:
            fx(0).wait()
            fx(1).start()
            cw_k.start()
            cw_q.wait()
            qproj(0)
            qproj(1)
            fx(1).wait()
            cw_v.start()
            cw_o.start()
            cw_k.wait()
            scores(0)
            qproj(2)
            scores(1)
            qproj(3)
            cw_v.wait()
            for c in copies(refs_a, 1, 1):
                c.start()
            cw_o.wait()
            pv(0)
            pv(1)
            scores(2)
            oproj(0)
            scores(3)
            oproj(1)
            pv(2)
            pv(3)
            oproj(2)
            oproj(3)
        else:
            qproj(0)
            qproj(1)
            scores(0)
            qproj(2)
            pv(0)
            scores(1)
            qproj(3)
            pv(1)
            scores(2)
            oproj(0)
            pv(2)
            scores(3)
            oproj(1)
            pv(3)
            oproj(2)
            oproj(3)

    @pl.when(s == 0)
    def _():
        step(True)

    @pl.when(s > 0)
    def _():
        step(False)

    @pl.when(s == NSTEPS - 1)
    def _():
        for br in range(2):
            for c in range(NCH):
                out_copy(br, c).wait()


@jax.jit
def pallas_concat_heads__mha_block_cached__mha_block_cached__near_ridge_kernel(
    A_x, A_k_cache, A_v_cache, A_wq, A_wo, B_x, B_k_cache, B_v_cache, B_wq, B_wo,
):
    bf = jnp.bfloat16
    any_spec = pl.BlockSpec(memory_space=pl.ANY)
    out = pl.pallas_call(
        _kernel,
        grid=(NSTEPS,),
        in_specs=[any_spec] * 10,
        out_specs=any_spec,
        out_shape=jax.ShapeDtypeStruct((M, 2 * D), bf),
        scratch_shapes=[
            pltpu.VMEM((2, M, D), bf),
            pltpu.VMEM((2, D, GW), bf),
            pltpu.VMEM((2, B, HPG, SK, DH), bf),
            pltpu.VMEM((2, B, HPG, SK, DH), bf),
            pltpu.VMEM((2, GW, D), bf),
            pltpu.VMEM((B, HPG, SQ, DH), bf),
            pltpu.VMEM((B, HPG * SQ, HPG * SK), bf),
            pltpu.VMEM((M, GW), bf),
            pltpu.VMEM((M, D), jnp.float32),
            pltpu.VMEM((2, M, D), bf),
            pltpu.SemaphoreType.DMA((1,)),
            pltpu.SemaphoreType.DMA((2,)),
            pltpu.SemaphoreType.DMA((2,)),
            pltpu.SemaphoreType.DMA((2,)),
            pltpu.SemaphoreType.DMA((2,)),
            pltpu.SemaphoreType.DMA((2, NCH)),
            pltpu.SemaphoreType.DMA((2,)),
        ],
        compiler_params=pltpu.CompilerParams(
            dimension_semantics=("arbitrary",),
            vmem_limit_bytes=64 * 1024 * 1024,
            disable_bounds_checks=True,
        ),
    )(A_x.reshape(M, D), A_k_cache, A_v_cache, A_wq, A_wo,
      B_x.reshape(M, D), B_k_cache, B_v_cache, B_wq, B_wo)
    return out.reshape(B, SQ, 2 * D)
```

```python
import jax
import jax.numpy as jnp
from jax import lax
import jax.experimental.pallas as pl
import jax.experimental.pallas.tpu as pltpu

B, SQ, D = 32, 32, 640
H, SK, DH = 32, 32, 128
M = B * SQ
HPG = 4
G = H // HPG
GW = HPG * DH
NSTEPS = 2 * G
SCALE = DH ** -0.5
NCH = 4
CB = B // NCH
CM = CB * SQ


def _kernel(xa, ka, va, wqa, woa, xb, kb, vb, wqb, wob, out_hbm,
            x_buf, wq_buf, k_buf, v_buf, wo_buf, q_scr, p_scr, o_scr, acc, out_buf,
            x_sem, wq_sem, k_sem, v_sem, wo_sem, out_sem, f_sem):
    s = pl.program_id(0)
    branch = s // G
    g = s % G
    slot = s % 2
    last_g = g == G - 1

    def copies(refs, gg, sl):
        k_h, v_h, wq_h, wo_h = refs
        return (
            pltpu.make_async_copy(wq_h.at[:, pl.ds(gg * GW, GW)], wq_buf.at[sl], wq_sem.at[sl]),
            pltpu.make_async_copy(k_h.at[:, pl.ds(gg * HPG, HPG)], k_buf.at[sl], k_sem.at[sl]),
            pltpu.make_async_copy(v_h.at[:, pl.ds(gg * HPG, HPG)], v_buf.at[sl], v_sem.at[sl]),
            pltpu.make_async_copy(wo_h.at[pl.ds(gg * GW, GW), :], wo_buf.at[sl], wo_sem.at[sl]),
        )

    def out_copy(br, c):
        return pltpu.make_async_copy(
            out_buf.at[br, pl.ds(c * CM, CM), :],
            out_hbm.at[pl.ds(c * CM, CM), pl.ds(br * D, D)],
            out_sem.at[br, c])

    def fx(c):
        return pltpu.make_async_copy(xa.at[pl.ds(c * (M // 2), M // 2), :],
                                     x_buf.at[0, pl.ds(c * (M // 2), M // 2), :], f_sem.at[c])

    def xb_copy():
        return pltpu.make_async_copy(xb, x_buf.at[1], x_sem.at[0])

    refs_a = (ka, va, wqa, woa)
    refs_b = (kb, vb, wqb, wob)

    def step(first):
        cw_q, cw_k, cw_v, cw_o = copies(refs_a, 0, slot)
        if first:
            fx(0).start()
            cw_q.start()
            acc[...] = jnp.zeros_like(acc)
        else:
            @pl.when(s == G)
            def _():
                xb_copy().wait()

            cw_q.wait()
            cw_k.wait()
            cw_v.wait()
            cw_o.wait()

            nxt = s + 1

            @pl.when(nxt < G)
            def _():
                for c in copies(refs_a, nxt, 1 - slot):
                    c.start()

            @pl.when(jnp.logical_and(nxt >= G, nxt < NSTEPS))
            def _():
                for c in copies(refs_b, nxt - G, 1 - slot):
                    c.start()

            @pl.when(s == 1)
            def _():
                xb_copy().start()

        row = lax.broadcasted_iota(jnp.int32, (HPG * SQ, HPG * SK), 0) // SQ
        col = lax.broadcasted_iota(jnp.int32, (HPG * SQ, HPG * SK), 1) // SK
        mask = row == col

        def qproj(c):
            x = x_buf[branch, c * CM:(c + 1) * CM, :]
            for h in range(HPG):
                qh = jnp.dot(x, wq_buf[slot, :, h * DH:(h + 1) * DH],
                             preferred_element_type=jnp.float32)
                q_scr[c * CB:(c + 1) * CB, h] = qh.astype(jnp.bfloat16).reshape(CB, SQ, DH)

        def scores(c):
            for b in range(c * CB, (c + 1) * CB):
                qs = q_scr[b].reshape(HPG * SQ, DH)
                ks = k_buf[slot, b].reshape(HPG * SK, DH)
                sc = lax.dot_general(qs, ks, (((1,), (1,)), ((), ())),
                                     preferred_element_type=jnp.float32)
                sc = jnp.where(mask, sc, -jnp.inf)
                m = jnp.max(sc, axis=1, keepdims=True)
                e = jnp.exp((sc - m) * SCALE)
                l = jnp.sum(e, axis=1, keepdims=True)
                r0 = pl.reciprocal(l, approx=True)
                r = r0 * (2.0 - l * r0)
                p_scr[b] = (e * r).astype(jnp.bfloat16)

        def pv(c):
            for b in range(c * CB, (c + 1) * CB):
                vs = v_buf[slot, b].reshape(HPG * SK, DH)
                o = jnp.dot(p_scr[b], vs, preferred_element_type=jnp.float32).astype(jnp.bfloat16)
                for h in range(HPG):
                    o_scr[b * SQ:(b + 1) * SQ, h * DH:(h + 1) * DH] = o[h * SQ:(h + 1) * SQ, :]

        def oproj(c):
            a = acc[c * CM:(c + 1) * CM, :] + jnp.dot(o_scr[c * CM:(c + 1) * CM, :], wo_buf[slot],
                                                      preferred_element_type=jnp.float32)
            if first:
                acc[c * CM:(c + 1) * CM, :] = a
            else:
                out_buf[branch, c * CM:(c + 1) * CM, :] = a.astype(jnp.bfloat16)
                acc[c * CM:(c + 1) * CM, :] = jnp.where(last_g, 0.0, a)

                @pl.when(last_g)
                def _():
                    out_copy(branch, c).start()

        if first:
            fx(0).wait()
            fx(1).start()
            cw_k.start()
            cw_q.wait()
            qproj(0)
            qproj(1)
            fx(1).wait()
            cw_v.start()
            cw_o.start()
            cw_k.wait()
            scores(0)
            qproj(2)
            scores(1)
            qproj(3)
            cw_v.wait()
            for c in copies(refs_a, 1, 1):
                c.start()
            cw_o.wait()
            pv(0)
            pv(1)
            scores(2)
            oproj(0)
            scores(3)
            oproj(1)
            pv(2)
            pv(3)
            oproj(2)
            oproj(3)
        else:
            qproj(0)
            qproj(1)
            scores(0)
            qproj(2)
            pv(0)
            scores(1)
            qproj(3)
            pv(1)
            scores(2)
            oproj(0)
            pv(2)
            scores(3)
            oproj(1)
            pv(3)
            oproj(2)
            oproj(3)

    @pl.when(s == 0)
    def _():
        step(True)

    @pl.when(s > 0)
    def _():
        step(False)

    @pl.when(s == NSTEPS - 1)
    def _():
        for br in range(2):
            for c in range(NCH):
                out_copy(br, c).wait()


@jax.jit
def pallas_concat_heads__mha_block_cached__mha_block_cached__near_ridge_kernel(
    A_x, A_k_cache, A_v_cache, A_wq, A_wo, B_x, B_k_cache, B_v_cache, B_wq, B_wo,
):
    bf = jnp.bfloat16
    any_spec = pl.BlockSpec(memory_space=pl.ANY)
    out = pl.pallas_call(
        _kernel,
        grid=(NSTEPS,),
        in_specs=[any_spec] * 10,
        out_specs=any_spec,
        out_shape=jax.ShapeDtypeStruct((M, 2 * D), bf),
        scratch_shapes=[
            pltpu.VMEM((2, M, D), bf),
            pltpu.VMEM((2, D, GW), bf),
            pltpu.VMEM((2, B, HPG, SK, DH), bf),
            pltpu.VMEM((2, B, HPG, SK, DH), bf),
            pltpu.VMEM((2, GW, D), bf),
            pltpu.VMEM((B, HPG, SQ, DH), bf),
            pltpu.VMEM((B, HPG * SQ, HPG * SK), bf),
            pltpu.VMEM((M, GW), bf),
            pltpu.VMEM((M, D), jnp.float32),
            pltpu.VMEM((2, M, D), bf),
            pltpu.SemaphoreType.DMA((1,)),
            pltpu.SemaphoreType.DMA((2,)),
            pltpu.SemaphoreType.DMA((2,)),
            pltpu.SemaphoreType.DMA((2,)),
            pltpu.SemaphoreType.DMA((2,)),
            pltpu.SemaphoreType.DMA((2, NCH)),
            pltpu.SemaphoreType.DMA((2,)),
        ],
        compiler_params=pltpu.CompilerParams(
            dimension_semantics=("arbitrary",),
            vmem_limit_bytes=64 * 1024 * 1024,
            disable_bounds_checks=True,
        ),
    )(A_x.reshape(M, D), A_k_cache, A_v_cache, A_wq, A_wo,
      B_x.reshape(M, D), B_k_cache, B_v_cache, B_wq, B_wo)
    return out.reshape(B, SQ, 2 * D)
```
